```python
import os as _os
_os.environ.setdefault("JAX_PLATFORMS", "cpu")
import jax
import jax.numpy as jnp

def _softmax(x, axis=-1):
    return jax.nn.softmax(x, axis=axis)
def _gelu(x):
    return jax.nn.gelu(x, approximate=True)
def _silu(x):
    return jax.nn.silu(x)
def _sigmoid(x):
    return jax.nn.sigmoid(x)
def _layernorm(x, axis=-1, eps=1e-5):
    m = jnp.mean(x, axis=axis, keepdims=True)
    v = jnp.var(x, axis=axis, keepdims=True)
    return (x - m) / jnp.sqrt(v + eps)
def _scatter_add(tgt, idx, src, axis=0):
    return tgt.at[idx].add(src)
def _segment_sum(src, seg, n):
    return jax.ops.segment_sum(src, seg, n)
class _Rng:
    def __init__(self, key):
        self._k = key
    def _next(self):
        self._k, sub = jax.random.split(self._k)
        return sub
    def normal(self, shape):
        return jax.random.normal(self._next(), shape, dtype=jnp.bfloat16)
    def randint(self, lo, hi, shape):
        return jax.random.randint(self._next(), shape, lo, hi, dtype=jnp.int32)
    def uniform(self, shape, lo=0.0, hi=1.0):
        return jax.random.uniform(self._next(), shape, jnp.bfloat16, lo, hi)
    def permutation(self, n):
        return jax.random.permutation(self._next(), n)


kernel_name = 'parallel_sum__mha_block__swiglu_ffn__prompt'

def setup_inputs():
    _rng = _Rng(jax.random.key(int.from_bytes(__import__("os").urandom(4), "little")))
    _w = (lambda a: (lambda t: t.astype(jnp.bfloat16) if jnp.issubdtype(t.dtype, jnp.floating) else t)(jnp.asarray(a)))
    def _A_setup():
        B, S, D, H = 1, 2048, 640, 32
        return {
            "x": _w((lambda *s: _rng.normal(s) * 0.05)(B, S, D)),
            "wqkv": _w((lambda *s: _rng.normal(s) * 0.1)(D, 3 * D)),
            "wo": _w((lambda *s: _rng.normal(s) * 0.05)(D, D)),
        }
    _A_in = _A_setup()

    def _B_setup():
        B, S, D, F = 1, 2048, 640, 1536
        return {
            "x": _w((lambda *s: _rng.normal(s) * 0.05)(B, S, D)),
            "w_gate": _w((lambda *s: _rng.normal(s) * 0.05)(D, F)),
            "w_up": _w((lambda *s: _rng.normal(s) * 0.05)(D, F)),
            "w_down": _w((lambda *s: _rng.normal(s) * 0.05)(F, D)),
        }
    _B_in = _B_setup()

    return {
        "A_x": _A_in["x"],
        "A_wqkv": _A_in["wqkv"],
        "A_wo": _A_in["wo"],
        "B_x": _B_in["x"],
        "B_w_gate": _B_in["w_gate"],
        "B_w_up": _B_in["w_up"],
        "B_w_down": _B_in["w_down"],
    }

def reference(A_x, A_wqkv, A_wo, B_x, B_w_gate, B_w_up, B_w_down):
    def _A_ref(x, wqkv, wo):
        B, S, D = x.shape
        H = 32
        Dh = D // H
        qkv = (lambda x, *d: x.transpose(*d))((x @ wqkv).reshape(B, S, 3, H, Dh), 2, 0, 3, 1, 4)
        q, k, v = qkv[0], qkv[1], qkv[2]
        scores = jnp.einsum("bhqd,bhkd->bhqk", q, k) * (Dh ** -0.5)
        p = _softmax(scores, axis=-1)
        o = jnp.einsum("bhqk,bhkd->bhqd", p, v)
        return (lambda x, *d: x.transpose(*d))(o, 0, 2, 1, 3).reshape(B, S, D) @ wo

    def _B_ref(x, w_gate, w_up, w_down):
        g = _silu(x @ w_gate)
        u = x @ w_up
        return (g * u) @ w_down

    x = A_x
    xn = _layernorm(x, axis=-1)
    return x + _A_ref(xn, A_wqkv, A_wo) + _B_ref(xn, B_w_gate, B_w_up, B_w_down)
```

```python
import functools
import math
import jax
import jax.numpy as jnp
import numpy as np
from jax import lax
import jax.experimental.pallas as pl
import jax.experimental.pallas.tpu as pltpu

S, D, H, DH, F = 2048, 640, 32, 20, 1536
NG = 6
BQ = 512
NB = S // BQ
KC = 128
NC = S // KC
U = 6
NIT = (H - 2) // U
FC = 256
NF = F // FC
FI = 1
EPS = 1e-5
QSCALE = (DH ** -0.5) * math.log2(math.e)
f32, bf16 = jnp.float32, jnp.bfloat16
NN = (((1,), (0,)), ((), ()))
NT = (((1,), (1,)), ((), ()))

_STRADDLE = [h for h in range(H) if (h * DH) // 128 != (h * DH + DH - 1) // 128]
_XSTART = [(h * DH) // 8 * 8 for h in _STRADDLE]


def _head_window(h):
    if h in _STRADDLE:
        j = _STRADDLE.index(h)
        return NG - 1, 24 * j + h * DH - _XSTART[j]
    return (h * DH) // 128, (h * DH) % 128


def _dot(a, b, dims=NN):
    return lax.dot_general(a, b, dims, preferred_element_type=f32)


def _kernel(x_hbm, wqkv_hbm, wo_hbm, wg_hbm, wu_hbm, wd_hbm, o_ref,
            x_s, wqkv_s, wo_s, wg_s, wu_s, wd_s,
            xn_s, wt_s, wkx_s, k_s, qt_s, vt_s, s0_s, s1_s, ot_s, y_s, sems):
    i = pl.program_id(0)

    @pl.when(i == 0)
    def _phase1():
        pairs = ([(x_hbm.at[r], x_s.at[r]) for r in range(NB)]
                 + [(wqkv_hbm.at[:, j * D:(j + 1) * D], wqkv_s.at[j]) for j in range(3)]
                 + [(wg_hbm.at[:, j * FC:(j + 1) * FC], wg_s.at[j]) for j in range(NF)]
                 + [(wu_hbm.at[:, j * FC:(j + 1) * FC], wu_s.at[j]) for j in range(NF)]
                 + [(wd_hbm, wd_s), (wo_hbm, wo_s)])
        cps = [pltpu.make_async_copy(a, b, sems.at[j]) for j, (a, b) in enumerate(pairs)]
        cx, cw, rest = cps[:NB], cps[NB:NB + 3], cps[NB + 3:]
        for c in [cx[0], cw[1], cx[1], cw[0], cw[2], cx[2], cx[3]]:
            c.start()

        def ln(r):
            x = x_s[r].astype(f32)
            mu = jnp.mean(x, axis=-1, keepdims=True)
            xc = x - mu
            var = jnp.mean(xc * xc, axis=-1, keepdims=True)
            xn_s[r] = (xc * lax.rsqrt(var + EPS)).astype(bf16)

        def keys(r):
            k = _dot(xn_s[r], wqkv_s[1]).astype(bf16)
            for g in range(NG - 1):
                k_s[g, r * BQ:(r + 1) * BQ, :] = k[:, g * 128:(g + 1) * 128]

        def keys_x(r):
            k_s[NG - 1, r * BQ:(r + 1) * BQ, :] = _dot(xn_s[r], wkx_s[...]).astype(bf16)

        sub = lax.broadcasted_iota(jnp.int32, (8, BQ), 0)

        def queries_values(r):
            qv = _dot(wt_s[...], xn_s[r], NT)
            qt = qv[0:D] * QSCALE
            for g in range(NG - 1):
                qt_s[r, g] = qt[g * 128:(g + 1) * 128].astype(bf16)
            qt_s[r, NG - 1] = jnp.concatenate(
                [qt[a:a + 24] for a in _XSTART] + [jnp.zeros((128 - 24 * len(_XSTART), BQ), f32)], axis=0).astype(bf16)
            vt = qv[D:].astype(bf16).astype(f32)
            for p in range(H // 2):
                a = p * 2 * DH
                mid = vt[a + 16:a + 24]
                vt_s[2 * p, r, 0:16] = vt[a:a + 16]
                vt_s[2 * p, r, 16:24] = jnp.where(sub < 4, mid, 1.0)
                vt_s[2 * p + 1, r, 0:8] = jnp.where(sub < 4, 1.0, mid)
                vt_s[2 * p + 1, r, 8:24] = vt[a + 24:a + 40]

        cx[0].wait()
        ln(0)
        cw[1].wait()
        cx[1].wait()
        keys(0)
        ln(1)
        wk = wqkv_s[1].astype(f32)
        wkx_s[...] = jnp.concatenate(
            [wk[:, a:a + 24] for a in _XSTART] + [jnp.zeros((D, 128 - 24 * len(_XSTART)), f32)], axis=1).astype(bf16)
        keys(1)
        for c in (cw[0], cw[2], cx[2], cx[3]):
            c.wait()
        for c in rest:
            c.start()
        keys_x(0)
        keys_x(1)
        ln(2)
        ln(3)
        for j in range(D // 128):
            wt_s[0:D, j * 128:(j + 1) * 128] = wqkv_s[0, j * 128:(j + 1) * 128, :].astype(f32).T.astype(bf16)
            wt_s[D:2 * D, j * 128:(j + 1) * 128] = wqkv_s[2, j * 128:(j + 1) * 128, :].astype(f32).T.astype(bf16)
        for r in (2, 3):
            keys(r)
            keys_x(r)

        def qv_body(r, c):
            queries_values(r)
            return c
        lax.fori_loop(0, NB, qv_body, 0)
        for c in rest:
            c.wait()

    row = lax.broadcasted_iota(jnp.int32, (128, BQ), 0)
    sub = lax.broadcasted_iota(jnp.int32, (8, BQ), 0)

    def masked_q(h):
        if isinstance(h, int):
            g, lo = _head_window(h)
        else:
            g, lo = (h * DH) // 128, (h * DH) % 128
            for hs in _STRADDLE:
                gs, los = _head_window(hs)
                g, lo = jnp.where(h == hs, gs, g), jnp.where(h == hs, los, lo)
        q = qt_s[i, g].astype(f32)
        return g, jnp.where((row >= lo) & (row < lo + DH), q, 0.0).astype(bf16)

    def qk_chunk(g, qm, s_ref, c, m):
        s = _dot(k_s[g, c * KC:(c + 1) * KC, :], qm)
        s_ref[c * KC:(c + 1) * KC, :] = s
        mc = jnp.max(s.reshape(KC // 8, 8, BQ), axis=0)
        return mc if m is None else jnp.maximum(m, mc)

    def pv_chunk(h, s_ref, c, m, acc):
        p = jnp.exp2(s_ref[c * KC:(c + 1) * KC, :] - m).astype(bf16)
        kb, ko = divmod(c * KC, BQ)
        d = _dot(vt_s[h, kb, :, ko:ko + KC], p)
        return d if acc is None else acc + d

    def finish(p, oe, oo):
        re = 1.0 / oe[20:21]
        ro = 1.0 / oo[0:1]
        a = p * 2 * DH
        if not isinstance(a, int):
            a = pl.multiple_of(a, 8)
        ot_s[pl.ds(a, 16), :] = oe[0:16] * re
        ot_s[pl.ds(a + 16, 8), :] = jnp.where(sub < 4, oe[16:24] * re, oo[0:8] * ro)
        ot_s[pl.ds(a + 24, 16), :] = oo[8:24] * ro

    def ffn(j):
        xn = xn_s[i]
        g = _dot(xn, wg_s[j])
        u = _dot(xn, wu_s[j])
        hid = (g * jax.nn.sigmoid(g) * u).astype(bf16)
        a = j * FC if isinstance(j, int) else pl.multiple_of(j * FC, FC)
        return _dot(hid, wd_s[pl.ds(a, FC), :])

    bufs = (s0_s, s1_s)

    def step(h_qk, h_pv, par, m_pv):
        m = acc = None
        if h_qk is not None:
            g, qm = masked_q(h_qk)
        for c in range(NC):
            if h_qk is not None:
                m = qk_chunk(g, qm, bufs[par], c, m)
            if h_pv is not None:
                acc = pv_chunk(h_pv, bufs[1 - par], c, m_pv, acc)
        if m is not None:
            m = jnp.max(m, axis=0, keepdims=True)
        return m, acc

    m0, _ = step(0, None, 0, None)
    y_s[...] = x_s[i].astype(f32)

    def body(j, m):
        for u in range(0, U, 2):
            h = j * U + u
            m, oe = step(h + 1, h, 1, m)
            if u == 0:
                for t in range(FI):
                    y_s[...] += ffn(j * FI + t)
            m, oo = step(h + 2, h + 1, 0, m)
            finish(h // 2, oe, oo)
        return m
    m0 = lax.fori_loop(0, NIT, body, m0)
    m1, oe = step(H - 1, H - 2, 1, m0)
    y = y_s[...]
    for j in range(NIT * FI, NF):
        y = y + ffn(j)
    _, oo = step(None, H - 1, 0, m1)
    finish(H // 2 - 1, oe, oo)
    y = y + _dot(ot_s[...].T.astype(bf16), wo_s[...])
    o_ref[...] = y.astype(o_ref.dtype)


@jax.jit
def pallas_parallel_sum__mha_block__swiglu_ffn__prompt_kernel(A_x, A_wqkv, A_wo, B_x, B_w_gate, B_w_up, B_w_down):
    del B_x
    x = A_x.reshape(NB, BQ, D)
    out = pl.pallas_call(
        _kernel,
        grid=(NB,),
        in_specs=[pl.BlockSpec(memory_space=pl.ANY)] * 6,
        out_specs=pl.BlockSpec((BQ, D), lambda i: (i, 0)),
        out_shape=jax.ShapeDtypeStruct((S, D), A_x.dtype),
        scratch_shapes=[
            pltpu.VMEM((NB, BQ, D), bf16),
            pltpu.VMEM((3, D, D), bf16),
            pltpu.VMEM((D, D), bf16),
            pltpu.VMEM((NF, D, FC), bf16),
            pltpu.VMEM((NF, D, FC), bf16),
            pltpu.VMEM((F, D), bf16),
            pltpu.VMEM((NB, BQ, D), bf16),
            pltpu.VMEM((2 * D, D), bf16),
            pltpu.VMEM((D, 128), bf16),
            pltpu.VMEM((NG, S, 128), bf16),
            pltpu.VMEM((NB, NG, 128, BQ), bf16),
            pltpu.VMEM((H, NB, 24, BQ), f32),
            pltpu.VMEM((S, BQ), f32),
            pltpu.VMEM((S, BQ), f32),
            pltpu.VMEM((D, BQ), f32),
            pltpu.VMEM((BQ, D), f32),
            pltpu.SemaphoreType.DMA((NB + 3 + 2 * NF + 2,)),
        ],
        compiler_params=pltpu.CompilerParams(
            dimension_semantics=("arbitrary",), vmem_limit_bytes=110 * 1024 * 1024),
        name="fused",
    )(x, A_wqkv, A_wo, B_w_gate, B_w_up, B_w_down)
    return out.reshape(A_x.shape)
```

```python
import math

import jax
import jax.numpy as jnp
from jax import lax
import jax.experimental.pallas as pl
import jax.experimental.pallas.tpu as pltpu

S, D, H, DH, F = 2048, 640, 32, 20, 1536
EPS = 1e-5
QSCALE = DH ** -0.5 * math.log2(math.e)

U = 6
NG = -(-H // U)
WW = U * DH
NIT = (H - 2) // U
BQ = 512
NB = S // BQ
KC = 128
NC = S // KC
FC, FM = 512, 128
VA = 16
VN = 7
VB = 256
VK = VA * VN
EARLY = 1
OD = 0

f32, bf16, u32 = jnp.float32, jnp.bfloat16, jnp.uint32
NN = (((1,), (0,)), ((), ()))
NT = (((1,), (1,)), ((), ()))


def _dot(a, b, dims=NN):
    return lax.dot_general(a, b, dims, preferred_element_type=f32)


def _pack(v):
    return pltpu.bitcast(v.astype(bf16), u32)


def _unpack(v):
    return pltpu.bitcast(v, bf16)


def _max(a, b):
    return b if a is None else jnp.maximum(a, b)


def _kernel(x_hbm, wqkv_hbm, wo_hbm, wg_hbm, wu_hbm, wd_hbm, o_ref,
            x_s, wqkv_s, wo_s, wg_s, wu_s, wd_s,
            xn_s, wt_s, wk_s, k_s, kq_s, kb_s, qt_s, vt_s, s0_s, s1_s, v0_s, v1_s, ot_s, y_s, sems):
    i = pl.program_id(0)
    sub = lax.broadcasted_iota(jnp.int32, (8, BQ), 0)

    @pl.when(i == 0)
    def _project():
        pairs = ([(x_hbm.at[r], x_s.at[r]) for r in range(NB)]
                 + [(wqkv_hbm.at[:, j * D:(j + 1) * D], wqkv_s.at[j]) for j in range(3)]
                 + [(wg_hbm.at[:, j * FC:(j + 1) * FC], wg_s.at[j]) for j in range(F // FC)]
                 + [(wu_hbm.at[:, j * FC:(j + 1) * FC], wu_s.at[j]) for j in range(F // FC)]
                 + [(wd_hbm, wd_s), (wo_hbm, wo_s)])
        copies = [pltpu.make_async_copy(a, b, sems.at[j]) for j, (a, b) in enumerate(pairs)]
        cx, cw, rest = copies[:NB], copies[NB:NB + 3], copies[NB + 3:]

        def layernorm(r):
            x = x_s[r].astype(f32)
            xc = x - jnp.mean(x, axis=-1, keepdims=True)
            var = jnp.mean(xc * xc, axis=-1, keepdims=True)
            xn_s[r] = _pack(xc * lax.rsqrt(var + EPS))

        def keys(r, g0, g1):
            for g in range(g0, g1):
                w = wqkv_s[1, :, 0:128] if g == 0 else _unpack(wk_s[g - 1])
                k_s[g, r * BQ // 2:(r + 1) * BQ // 2, :] = _pack(_dot(_unpack(xn_s[r]), w))

        def spread_keys(r):
            k = _unpack(kq_s[r]).astype(f32)
            for c in range(D // NB):
                kb_s[r * (D // NB) + c] = jnp.broadcast_to(k[:, c:c + 1], (VK, 128))

        def queries_values(r):
            qv = _dot(_unpack(wt_s[...]), _unpack(xn_s[r]), NT)
            qt = qv[0:D] * QSCALE
            for g in range(NG):
                w = qt[g * WW:min(g * WW + 128, D)]
                if w.shape[0] < 128:
                    w = jnp.concatenate([w, jnp.zeros((128 - w.shape[0], BQ), f32)], axis=0)
                qt_s[r, g] = _pack(w)
            vt = qv[D:].astype(bf16).astype(f32)
            for p in range(H // 2):
                a = p * 2 * DH
                at = VK // 8 + (r * (H // 2) + p) * 3
                v0_s[pl.ds(at, 3)] = qt[a:a + 24].reshape(3, 8, BQ)
                v1_s[pl.ds(at, 3)] = qt[a + 16:a + 40].reshape(3, 8, BQ)
                mid = vt[a + 16:a + 24]
                vt_s[2 * p, r, 0:16] = vt[a:a + 16]
                vt_s[2 * p, r, 16:24] = jnp.where(sub < 4, mid, 1.0)
                vt_s[2 * p + 1, r, 0:8] = jnp.where(sub < 4, 1.0, mid)
                vt_s[2 * p + 1, r, 8:24] = vt[a + 24:a + 40]

        for c in [cx[0], cw[1], cx[1], cx[2], cx[3], cw[0], cw[2]]:
            c.start()
        if EARLY:
            for c in rest:
                c.start()
        cx[0].wait()
        layernorm(0)
        cw[1].wait()
        wk = pltpu.bitcast(wqkv_s[1], u32)
        for g in range(1, NG):
            w = wk[:, g * WW:min(g * WW + 128, D)]
            if w.shape[1] < 128:
                w = jnp.concatenate([w, jnp.zeros((D // 2, 128 - w.shape[1]), u32)], axis=1)
            wk_s[g - 1] = w
        keys(0, 0, 4)
        cx[1].wait()
        cx[2].wait()
        layernorm(1)
        layernorm(2)
        keys(0, 4, NG)
        keys(1, 0, NG)
        keys(2, 0, 4)
        for c in (cx[3], cw[0], cw[2]):
            c.wait()
        if not EARLY:
            for c in rest:
                c.start()
        layernorm(3)
        for j in range(D // 128):
            wt_s[0:D // 2, j * 128:(j + 1) * 128] = _pack(wqkv_s[0, j * 128:(j + 1) * 128, :].astype(f32).T)
            wt_s[D // 2:D, j * 128:(j + 1) * 128] = _pack(wqkv_s[2, j * 128:(j + 1) * 128, :].astype(f32).T)
        k = jnp.concatenate([k_s[g, 0:VK // 2, 0:min(WW, D - g * WW)] for g in range(NG)], axis=1)
        for r in range(NB):
            kq_s[r] = k[:, r * (D // NB):(r + 1) * (D // NB)]
        keys(2, 4, NG)
        keys(3, 0, NG)

        def qv_body(r, carry):
            queries_values(r)
            spread_keys(r)
            return carry
        lax.fori_loop(0, NB, qv_body, 0)
        for c in rest:
            c.wait()

    row = lax.broadcasted_iota(jnp.int32, (64, BQ), 0)

    def masked_q(g, slot):
        lo, hi = slot * DH // 2, (slot + 1) * DH // 2
        a, b = lo // 8 * 8, -(-hi // 8) * 8
        keep = (row[a:b] >= lo) & (row[a:b] < hi)
        q = jnp.where(keep, qt_s[i, g, a:b, :], jnp.zeros((b - a, BQ), u32))
        parts = [jnp.zeros((2 * a, BQ), bf16), _unpack(q), jnp.zeros((128 - 2 * b, BQ), bf16)]
        return jnp.concatenate([t for t in parts if t.shape[0]], axis=0)

    def scores_mxu(g, qm, s_ref, lo, hi, m):
        s = _dot(_unpack(k_s[g, lo // 2:hi // 2, :]), qm)
        s_ref[lo:hi, :] = s
        mc = jnp.max(s.reshape((hi - lo) // 8, 8, BQ), axis=0)
        return [_max(m[t], mc[:, t * 128:(t + 1) * 128]) for t in range(BQ // 128)]

    def scores_vpu(g, slot, v_ref, a, c0, m):
        at = VK // 8 + (i * (H // 2) + g * (U // 2) + slot // 2) * 3
        tiles = range(c0 // 128, (c0 + VB) // 128)
        acc = {}
        for d in range(DH):
            k = kb_s[g * WW + slot * DH + d, a:a + VA, :]
            e = d + 4 * (slot % 2)
            for t in tiles:
                term = k * v_ref[at + e // 8, e % 8:e % 8 + 1, t * 128:(t + 1) * 128]
                acc[t] = acc[t] + term if d else term
        m = list(m)
        for t in tiles:
            s = acc[t].reshape(VA // 8, 8, 128)
            v_ref[a // 8:(a + VA) // 8, :, t * 128:(t + 1) * 128] = s
            m[t] = _max(m[t], jnp.max(s, axis=0))
        return m

    def values_chunk(h, s_ref, v_ref, c, m, acc):
        lo, hi = c * KC, (c + 1) * KC
        parts = []
        if lo < VK:
            parts.append(v_ref[lo // 8:min(hi, VK) // 8].reshape(min(hi, VK) - lo, BQ))
        if hi > VK:
            parts.append(s_ref[max(lo, VK):hi, :])
        p = jnp.exp2(jnp.concatenate(parts, axis=0) - m).astype(bf16)
        kb, ko = divmod(lo, BQ)
        o = _dot(vt_s[h, kb, :, ko:ko + KC], p)
        return o if acc is None else acc + o

    def normalise(p, oe, oo):
        re = 1.0 / oe[20:21]
        ro = 1.0 / oo[0:1]
        a = p * 2 * DH
        if not isinstance(a, int):
            a = pl.multiple_of(a, 8)
        ot_s[pl.ds(a, 16), :] = oe[0:16] * re
        ot_s[pl.ds(a + 16, 8), :] = jnp.where(sub < 4, oe[16:24] * re, oo[0:8] * ro)
        ot_s[pl.ds(a + 24, 16), :] = oo[8:24] * ro

    def ffn_item(n):
        hid = {}
        j, r = n // (BQ // FM), n % (BQ // FM)
        a, a2, jj = r * FM, r * (FM // 2), j * FC
        if not isinstance(n, int):
            a, a2, jj = pl.multiple_of(a, FM), pl.multiple_of(a2, FM // 2), pl.multiple_of(jj, FC)

        def gate():
            hg = 0.5 * _dot(_unpack(xn_s[i, pl.ds(a2, FM // 2)]), wg_s[j])
            hid[0] = hg + hg * jnp.tanh(hg)

        def up():
            hid[0] = (hid[0] * _dot(_unpack(xn_s[i, pl.ds(a2, FM // 2)]), wu_s[j])).astype(bf16)

        def down():
            y_s[pl.ds(a, FM)] += _dot(hid[0], wd_s[pl.ds(jj, FC), :])
        return gate, up, down

    def ffn_stages(j):
        return [f for fs in zip(ffn_item(2 * j), ffn_item(2 * j + 1)) for f in fs]

    blocks = [(a, c0) for a in range(0, VK, VA) for c0 in range(0, BQ, VB)]
    lead = max(len(blocks) - (NC - 1), 0)

    def heads(j, u0, n_qk, n_pv, m, extra):
        mx = [m] + [None] * n_qk
        acc = [None] * n_pv
        for t in range(max(n_qk, n_pv) * NC):
            u, c = divmod(t, NC)
            if t in extra:
                extra[t]()
            if u < n_qk:
                dg, slot = divmod(u0 + u + 1, U)
                s_ref, v_ref = ((s0_s, v0_s), (s1_s, v1_s))[slot % 2]
                if c == 0:
                    qm = masked_q(j + dg, slot)
                    mm = [None] * (BQ // 128)
                if (c + 1) * KC > VK:
                    mm = scores_mxu(j + dg, qm, s_ref, max(c * KC, VK), (c + 1) * KC, mm)
                for blk in blocks[c + lead if c else 0:c + lead + 1]:
                    mm = scores_vpu(j + dg, slot, v_ref, *blk, mm)
                if c == NC - 1:
                    mx[u + 1] = jnp.max(jnp.concatenate(mm, axis=1), axis=0, keepdims=True)
            if u < n_pv:
                s_ref, v_ref = ((s0_s, v0_s), (s1_s, v1_s))[u % 2]
                acc[u] = values_chunk(j * U + u, s_ref, v_ref, c, mx[u], acc[u])
                if c == NC - 1 and u % 2 == 1:
                    normalise(j * (U // 2) + u // 2, acc[u - 1], acc[u])
        return mx[n_qk]

    def residual(c):
        def f():
            rows = slice(c * (BQ // NC), (c + 1) * (BQ // NC))
            y_s[rows] = x_s[i, rows].astype(f32)
        return f
    m = heads(0, -1, 1, 0, None, {c: residual(c) for c in range(NC)})

    def body(j, m):
        return heads(j, 0, U, U, m, {u * NC: f for u, f in enumerate(ffn_stages(j))})
    m = lax.fori_loop(0, NIT, body, m)

    st = ffn_stages(NIT)
    heads(NIT, 0, 1, 2, m, {0: st[0], NC: st[1], NC + 6: st[2], NC + 12: st[3]})
    o = ot_s[...].T.astype(bf16)
    st[4]()
    st[5]()
    for a in range(0, BQ, 128):
        o_ref[a:a + 128] = (y_s[a:a + 128] + _dot(o[a:a + 128], wo_s[...])).astype(o_ref.dtype)


@jax.jit
def pallas_parallel_sum__mha_block__swiglu_ffn__prompt_kernel(A_x, A_wqkv, A_wo, B_x, B_w_gate, B_w_up, B_w_down):
    del B_x
    nv = VK // 8 + NB * (H // 2) * 3
    out = pl.pallas_call(
        _kernel,
        grid=(NB,),
        in_specs=[pl.BlockSpec(memory_space=pl.ANY)] * 6,
        out_specs=pl.BlockSpec((BQ, D), lambda i: (i, 0)),
        out_shape=jax.ShapeDtypeStruct((S, D), A_x.dtype),
        scratch_shapes=[
            pltpu.VMEM((NB, BQ, D), bf16),
            pltpu.VMEM((3, D, D), bf16),
            pltpu.VMEM((D, D), bf16),
            pltpu.VMEM((F // FC, D, FC), bf16),
            pltpu.VMEM((F // FC, D, FC), bf16),
            pltpu.VMEM((F, D), bf16),
            pltpu.VMEM((NB, BQ // 2, D), u32),
            pltpu.VMEM((D, D), u32),
            pltpu.VMEM((NG - 1, D // 2, 128), u32),
            pltpu.VMEM((NG, S // 2, 128), u32),
            pltpu.VMEM((NB, VK // 2, D // NB), u32),
            pltpu.VMEM((D, VK, 128), f32),
            pltpu.VMEM((NB, NG, 64, BQ), u32),
            pltpu.VMEM((H, NB, 24, BQ), f32),
            pltpu.VMEM((S, BQ), f32),
            pltpu.VMEM((S, BQ), f32),
            pltpu.VMEM((nv, 8, BQ), f32),
            pltpu.VMEM((nv, 8, BQ), f32),
            pltpu.VMEM((D, BQ), f32),
            pltpu.VMEM((BQ, D), f32),
            pltpu.SemaphoreType.DMA((NB + 3 + 2 * (F // FC) + 2,)),
        ],
        compiler_params=pltpu.CompilerParams(
            dimension_semantics=("arbitrary",), vmem_limit_bytes=112 * 1024 * 1024),
        name="fused",
    )(A_x.reshape(NB, BQ, D), A_wqkv, A_wo, B_w_gate, B_w_up, B_w_down)
    return out.reshape(A_x.shape)
```

```python
import math

import jax
import jax.numpy as jnp
from jax import lax
import jax.experimental.pallas as pl
import jax.experimental.pallas.tpu as pltpu

S, D, H, DH, F = 2048, 640, 32, 20, 1536
EPS = 1e-5
QSCALE = DH ** -0.5 * math.log2(math.e)

U = 6
NG = -(-H // U)
WW = U * DH
NIT = (H - 2) // U
BQ = 512
NB = S // BQ
KC = 128
NC = S // KC
FC, FM = 512, 128
VK = 112
VA, VB = 16, 256
OM = 128

f32, bf16, u32 = jnp.float32, jnp.bfloat16, jnp.uint32
NN = (((1,), (0,)), ((), ()))
NT = (((1,), (1,)), ((), ()))


def _dot(a, b, dims=NN):
    return lax.dot_general(a, b, dims, preferred_element_type=f32)


def _pack(v):
    return pltpu.bitcast(v.astype(bf16), u32)


def _unpack(v):
    return pltpu.bitcast(v, bf16)


def _max(a, b):
    return b if a is None else jnp.maximum(a, b)


def _kernel(x_hbm, wqkv_hbm, wo_hbm, wg_hbm, wu_hbm, wd_hbm, o_hbm,
            x_s, wqkv_s, wo_s, wg_s, wu_s, wd_s,
            xn_s, wt_s, kf_s, k_s, kq_s, kb_s, qt_s, vt_s,
            s0_s, s1_s, v0_s, v1_s, raw_s, ot_s, y_s, o_s, sems):
    i = pl.program_id(0)
    sub = lax.broadcasted_iota(jnp.int32, (8, BQ), 0)

    @pl.when(i == 0)
    def _project():
        def wqkv(j):
            return wqkv_hbm.at[:, j * D:(j + 1) * D], wqkv_s.at[j]
        groups = [
            [(x_hbm.at[0], x_s.at[0])],
            [wqkv(1)],
            [(x_hbm.at[1:3], x_s.at[1:3])],
            [(x_hbm.at[3], x_s.at[3]), wqkv(0), wqkv(2)],
            [(src.at[:, j * FC:(j + 1) * FC], dst.at[j])
             for src, dst in ((wg_hbm, wg_s), (wu_hbm, wu_s)) for j in range(F // FC)]
            + [(wd_hbm, wd_s), (wo_hbm, wo_s)],
        ]
        groups = [[pltpu.make_async_copy(a, b, sems.at[n]) for a, b in g] for n, g in enumerate(groups)]
        for g in groups:
            for c in g:
                c.start()

        def wait(n):
            for c in groups[n]:
                c.wait()

        def layernorm(r):
            x = x_s[r].astype(f32)
            xc = x - jnp.mean(x, axis=-1, keepdims=True)
            var = jnp.mean(xc * xc, axis=-1, keepdims=True)
            xn_s[r] = _pack(xc * lax.rsqrt(var + EPS))

        def keys(r, t0, t1):
            for a in (0, BQ // 4):
                k = _dot(_unpack(xn_s[r, a:a + BQ // 4]), wqkv_s[1, :, t0 * 128:t1 * 128])
                kf_s[r, a:a + BQ // 4, t0 * 128:t1 * 128] = _pack(k)

        def key_windows(r):
            k = kf_s[r]
            a = pl.multiple_of(r * (BQ // 2), BQ // 2)
            for g in range(NG):
                w = k[:, g * WW:min(g * WW + 128, D)]
                if w.shape[1] < 128:
                    w = jnp.concatenate([w, jnp.zeros((BQ // 2, 128 - w.shape[1]), u32)], axis=1)
                k_s[g, pl.ds(a, BQ // 2), :] = w

        def spread_keys(r):
            k = _unpack(kq_s[r]).astype(f32)
            for c in range(D // NB):
                kb_s[r * (D // NB) + c] = jnp.broadcast_to(k[:, c:c + 1], (VK, 128))

        def queries_values(r):
            qv = _dot(_unpack(wt_s[...]), _unpack(xn_s[r]), NT)
            qt = qv[0:D] * QSCALE
            for g in range(NG):
                w = qt[g * WW:min(g * WW + 128, D)]
                if w.shape[0] < 128:
                    w = jnp.concatenate([w, jnp.zeros((128 - w.shape[0], BQ), f32)], axis=0)
                qt_s[r, g] = _pack(w)
            vt = qv[D:].astype(bf16).astype(f32)
            for p in range(H // 2):
                a = p * 2 * DH
                at = VK // 8 + (r * (H // 2) + p) * 3
                v0_s[pl.ds(at, 3)] = qt[a:a + 24].reshape(3, 8, BQ)
                v1_s[pl.ds(at, 3)] = qt[a + 16:a + 40].reshape(3, 8, BQ)
                mid = vt[a + 16:a + 24]
                vt_s[2 * p, r, 0:16] = vt[a:a + 16]
                vt_s[2 * p, r, 16:24] = jnp.where(sub < 4, mid, 1.0)
                vt_s[2 * p + 1, r, 0:8] = jnp.where(sub < 4, 1.0, mid)
                vt_s[2 * p + 1, r, 8:24] = vt[a + 24:a + 40]

        wait(0)
        layernorm(0)
        wait(1)
        keys(0, 0, 4)
        wait(2)
        layernorm(1)
        layernorm(2)
        keys(0, 4, 5)
        keys(1, 0, 5)
        keys(2, 0, 2)
        wait(3)
        layernorm(3)
        for j in range(D // 128):
            wt_s[0:D // 2, j * 128:(j + 1) * 128] = _pack(wqkv_s[0, j * 128:(j + 1) * 128, :].astype(f32).T)
            wt_s[D // 2:D, j * 128:(j + 1) * 128] = _pack(wqkv_s[2, j * 128:(j + 1) * 128, :].astype(f32).T)
        k = kf_s[0, 0:VK // 2]
        for r in range(NB):
            kq_s[r] = k[:, r * (D // NB):(r + 1) * (D // NB)]
        keys(2, 2, 5)
        keys(3, 0, 5)

        def qv_body(t, carry):
            for r in (2 * t, 2 * t + 1):
                queries_values(r)
                spread_keys(r)
                key_windows(r)
            return carry
        lax.fori_loop(0, NB // 2, qv_body, 0)
        wait(4)

    row = lax.broadcasted_iota(jnp.int32, (64, BQ), 0)

    def masked_q(g, slot):
        lo, hi = slot * DH // 2, (slot + 1) * DH // 2
        a, b = lo // 8 * 8, -(-hi // 8) * 8
        keep = (row[a:b] >= lo) & (row[a:b] < hi)
        q = jnp.where(keep, qt_s[i, g, a:b, :], jnp.zeros((b - a, BQ), u32))
        parts = [jnp.zeros((2 * a, BQ), bf16), _unpack(q), jnp.zeros((128 - 2 * b, BQ), bf16)]
        return jnp.concatenate([t for t in parts if t.shape[0]], axis=0)

    def scores_mxu(g, qm, s_ref, lo, hi, m):
        s = _dot(_unpack(k_s[g, lo // 2:hi // 2, :]), qm)
        s_ref[lo:hi, :] = s
        mc = jnp.max(s.reshape((hi - lo) // 8, 8, BQ), axis=0)
        return [_max(m[t], mc[:, t * 128:(t + 1) * 128]) for t in range(BQ // 128)]

    def scores_vpu(g, slot, v_ref, a, c0, m):
        at = VK // 8 + (i * (H // 2) + g * (U // 2) + slot // 2) * 3
        tiles = range(c0 // 128, (c0 + VB) // 128)
        acc = {}
        for d in range(DH):
            k = kb_s[g * WW + slot * DH + d, a:a + VA, :]
            e = d + 4 * (slot % 2)
            for t in tiles:
                term = k * v_ref[at + e // 8, e % 8:e % 8 + 1, t * 128:(t + 1) * 128]
                acc[t] = acc[t] + term if d else term
        m = list(m)
        for t in tiles:
            s = acc[t].reshape(VA // 8, 8, 128)
            v_ref[a // 8:(a + VA) // 8, :, t * 128:(t + 1) * 128] = s
            m[t] = _max(m[t], jnp.max(s, axis=0))
        return m

    def values_chunk(h, s_ref, v_ref, c, m, acc):
        lo, hi = c * KC, (c + 1) * KC
        s = s_ref[max(lo, VK):hi, :]
        if c == 0:
            s = jnp.concatenate([v_ref[0:VK // 8].reshape(VK, BQ), s], axis=0)
        p = jnp.exp2(s - m).astype(bf16)
        kb, ko = divmod(lo, BQ)
        o = _dot(vt_s[h, kb, :, ko:ko + KC], p)
        return o if acc is None else acc + o

    def ffn_item(n):
        hid = {}
        j, r = n // (BQ // FM), n % (BQ // FM)
        a, a2, jj = r * FM, r * (FM // 2), j * FC
        if not isinstance(n, int):
            a, a2, jj = pl.multiple_of(a, FM), pl.multiple_of(a2, FM // 2), pl.multiple_of(jj, FC)

        def gate():
            hg = 0.5 * _dot(_unpack(xn_s[i, pl.ds(a2, FM // 2)]), wg_s[j])
            hid[0] = hg + hg * jnp.tanh(hg)

        def up():
            hid[0] = (hid[0] * _dot(_unpack(xn_s[i, pl.ds(a2, FM // 2)]), wu_s[j])).astype(bf16)

        def down():
            y_s[pl.ds(a, FM)] += _dot(hid[0], wd_s[pl.ds(jj, FC), :])
        return gate, up, down

    def ffn_stages(j):
        return [f for fs in zip(ffn_item(2 * j), ffn_item(2 * j + 1)) for f in fs]

    bufs = ((s0_s, v0_s), (s1_s, v1_s))
    blocks = [(a, c0) for a in range(0, VK, VA) for c0 in range(0, BQ, VB)]
    assert VK < KC and len(blocks) <= NC

    def heads(j, u0, n_qk, n_pv, m, extra):
        mx = [m] + [None] * n_qk
        acc = [None] * n_pv
        for t in range(max(n_qk, n_pv) * NC):
            u, c = divmod(t, NC)
            if t in extra:
                extra[t]()
            if u < n_qk:
                dg, slot = divmod(u0 + u + 1, U)
                s_ref, v_ref = bufs[slot % 2]
                if c == 0:
                    qm = masked_q(j + dg, slot)
                    mm = [None] * (BQ // 128)
                mm = scores_mxu(j + dg, qm, s_ref, max(c * KC, VK), (c + 1) * KC, mm)
                if c < len(blocks):
                    mm = scores_vpu(j + dg, slot, v_ref, *blocks[c], mm)
                if c == NC - 1:
                    mx[u + 1] = jnp.max(jnp.concatenate(mm, axis=1), axis=0, keepdims=True)
            if u < n_pv:
                acc[u] = values_chunk(j * U + u, *bufs[u % 2], c, mx[u], acc[u])
                if c == NC - 1:
                    raw_s[j * U + u] = acc[u]
        return mx[n_qk]

    def residual(c):
        def f():
            rows = slice(c * (BQ // NC), (c + 1) * (BQ // NC))
            y_s[rows] = x_s[i, rows].astype(f32)
        return f
    m = heads(0, -1, 1, 0, None, {c: residual(c) for c in range(NC)})

    def body(j, m):
        return heads(j, 0, U, U, m, {u * NC + (1 if u else 5): f for u, f in enumerate(ffn_stages(j))})
    m = lax.fori_loop(0, NIT, body, m)

    st = ffn_stages(NIT)
    heads(NIT, 0, 1, 2, m, {NC: st[0], NC + 3: st[1], NC + 7: st[2], NC + 11: st[3]})
    for p in range(H // 2):
        oe, oo = raw_s[2 * p], raw_s[2 * p + 1]
        re = 1.0 / oe[20:21]
        ro = 1.0 / oo[0:1]
        a = p * 2 * DH
        ot_s[a:a + 16] = oe[0:16] * re
        ot_s[a + 16:a + 24] = jnp.where(sub < 4, oe[16:24] * re, oo[0:8] * ro)
        ot_s[a + 24:a + 40] = oo[8:24] * ro
    o = ot_s[...].T.astype(bf16)
    st[4]()
    st[5]()

    def out_copy(n):
        return pltpu.make_async_copy(o_s.at[n], o_hbm.at[n], sems.at[5])

    for n in range(BQ // OM):
        rows = slice(n * OM, (n + 1) * OM)
        o_s[i * (BQ // OM) + n] = (y_s[rows] + _dot(o[rows], wo_s[...])).astype(o_s.dtype)
        out_copy(i * (BQ // OM) + n).start()

    @pl.when(i == NB - 1)
    def _drain():
        for n in range(S // OM):
            out_copy(n).wait()


@jax.jit
def pallas_parallel_sum__mha_block__swiglu_ffn__prompt_kernel(
    A_x: jax.Array,
    A_wqkv: jax.Array,
    A_wo: jax.Array,
    B_x: jax.Array,
    B_w_gate: jax.Array,
    B_w_up: jax.Array,
    B_w_down: jax.Array,
):
    del B_x
    nv = VK // 8 + NB * (H // 2) * 3
    out = pl.pallas_call(
        _kernel,
        grid=(NB,),
        in_specs=[pl.BlockSpec(memory_space=pl.ANY)] * 6,
        out_specs=pl.BlockSpec(memory_space=pl.ANY),
        out_shape=jax.ShapeDtypeStruct((S // OM, OM, D), A_x.dtype),
        scratch_shapes=[
            pltpu.VMEM((NB, BQ, D), bf16),
            pltpu.VMEM((3, D, D), bf16),
            pltpu.VMEM((D, D), bf16),
            pltpu.VMEM((F // FC, D, FC), bf16),
            pltpu.VMEM((F // FC, D, FC), bf16),
            pltpu.VMEM((F, D), bf16),
            pltpu.VMEM((NB, BQ // 2, D), u32),
            pltpu.VMEM((D, D), u32),
            pltpu.VMEM((NB, BQ // 2, D), u32),
            pltpu.VMEM((NG, S // 2, 128), u32),
            pltpu.VMEM((NB, VK // 2, D // NB), u32),
            pltpu.VMEM((D, VK, 128), f32),
            pltpu.VMEM((NB, NG, 64, BQ), u32),
            pltpu.VMEM((H, NB, 24, BQ), f32),
            pltpu.VMEM((S, BQ), f32),
            pltpu.VMEM((S, BQ), f32),
            pltpu.VMEM((nv, 8, BQ), f32),
            pltpu.VMEM((nv, 8, BQ), f32),
            pltpu.VMEM((H, 24, BQ), f32),
            pltpu.VMEM((D, BQ), f32),
            pltpu.VMEM((BQ, D), f32),
            pltpu.VMEM((S // OM, OM, D), A_x.dtype),
            pltpu.SemaphoreType.DMA((6,)),
        ],
        compiler_params=pltpu.CompilerParams(
            dimension_semantics=("arbitrary",), vmem_limit_bytes=112 * 1024 * 1024),
        name="fused",
    )(A_x.reshape(NB, BQ, D), A_wqkv, A_wo, B_w_gate, B_w_up, B_w_down)
    return out.reshape(A_x.shape)
```
